```python
import jax
import jax.numpy as jnp

def _softmax(x, axis=-1):
    return jax.nn.softmax(x, axis=axis)
def _gelu(x):
    return jax.nn.gelu(x, approximate=True)
def _silu(x):
    return jax.nn.silu(x)
def _sigmoid(x):
    return jax.nn.sigmoid(x)
def _layernorm(x, axis=-1, eps=1e-5):
    m = jnp.mean(x, axis=axis, keepdims=True)
    v = jnp.var(x, axis=axis, keepdims=True)
    return (x - m) / jnp.sqrt(v + eps)
def _scatter_add(tgt, idx, src, axis=0):
    return tgt.at[idx].add(src)
def _segment_sum(src, seg, n):
    return jax.ops.segment_sum(src, seg, n)
class _Rng:
    def __init__(self, key):
        self._k = key
    def _next(self):
        self._k, sub = jax.random.split(self._k)
        return sub
    def normal(self, shape):
        return jax.random.normal(self._next(), shape, dtype=jnp.bfloat16)
    def randint(self, lo, hi, shape):
        return jax.random.randint(self._next(), shape, lo, hi, dtype=jnp.int32)
    def uniform(self, shape, lo=0.0, hi=1.0):
        return jax.random.uniform(self._next(), shape, jnp.bfloat16, lo, hi)
    def permutation(self, n):
        return jax.random.permutation(self._next(), n)


kernel_name = 'sequential_preLN__spectral_gfnet__swiglu_ffn__prompt'

def _fwd_setup_inputs():
    _rng = _Rng(jax.random.key(int.from_bytes(__import__("os").urandom(4), "little")))
    _w = (lambda a: (lambda t: t.astype(jnp.bfloat16) if jnp.issubdtype(t.dtype, jnp.floating) else t)(jnp.asarray(a)))
    def _A_setup():
        B, S, D = 1, 2048, 576
        Df = D // 2 + 1
        return {
            "x": _w((lambda *s: _rng.normal(s) * 0.05)(B, S, D)),
            "w_r": _w((lambda *s: _rng.normal(s) * 0.05)(S, Df) * 0.02),
            "w_i": _w((lambda *s: _rng.normal(s) * 0.05)(S, Df) * 0.02),
        }
    _A_in = _A_setup()

    def _B_setup():
        B, S, D, F = 1, 2048, 576, 4608
        return {
            "x": _w((lambda *s: _rng.normal(s) * 0.05)(B, S, D)),
            "w_gate": _w((lambda *s: _rng.normal(s) * 0.05)(D, F)),
            "w_up": _w((lambda *s: _rng.normal(s) * 0.05)(D, F)),
            "w_down": _w((lambda *s: _rng.normal(s) * 0.05)(F, D)),
        }
    _B_in = _B_setup()

    return {
        "A_x": _A_in["x"],
        "A_w_r": _A_in["w_r"],
        "A_w_i": _A_in["w_i"],
        "B_x": _B_in["x"],
        "B_w_gate": _B_in["w_gate"],
        "B_w_up": _B_in["w_up"],
        "B_w_down": _B_in["w_down"],
    }

def _fwd_reference(A_x, A_w_r, A_w_i, B_x, B_w_gate, B_w_up, B_w_down):
    def _A_ref(x, w_r, w_i):
        B, S, D = x.shape
        X = (lambda x, axes=(-2,-1): jnp.fft.rfft2(x.astype(jnp.float32), axes=axes))(x, axes=(-2, -1))
        W = w_r + 1j * w_i
        X = X * W
        y = (lambda x, s, axes=(-2,-1): jnp.fft.irfft2(x, s=s, axes=axes).astype(jnp.bfloat16))(X, (S, D), axes=(-2, -1))
        return y

    def _B_ref(x, w_gate, w_up, w_down):
        g = _silu(x @ w_gate)
        u = x @ w_up
        return (g * u) @ w_down

    x = A_x
    h = x + _A_ref(_layernorm(x, axis=-1), A_w_r, A_w_i)
    h2 = h + _B_ref(_layernorm(h, axis=-1), B_w_gate, B_w_up, B_w_down)
    return h2


def setup_inputs():
    _inp = _fwd_setup_inputs()
    _gk = jax.random.fold_in(jax.random.key(int.from_bytes(__import__("os").urandom(4), "little")), 2**31 - 1)
    _shapes = [[1, 2048, 576]]
    _dtypes = ['bfloat16']
    _gks = jax.random.split(_gk, len(_shapes))
    _gs = [jax.random.normal(k, s, dtype=jnp.dtype(d)) * 0.05 for k, s, d in zip(_gks, _shapes, _dtypes)]
    _inp["grad_out"] = _gs[0]
    return _inp

def reference(A_x, A_w_r, A_w_i, B_w_gate, B_w_up, B_w_down, B_x, grad_out):
    _const = dict(B_x=B_x)
    def _f(*_d):
        return _fwd_reference(**{'A_x': _d[0], 'A_w_r': _d[1], 'A_w_i': _d[2], 'B_w_gate': _d[3], 'B_w_up': _d[4], 'B_w_down': _d[5], **_const})
    _out, _vjp = jax.vjp(_f, A_x, A_w_r, A_w_i, B_w_gate, B_w_up, B_w_down)
    _grads = _vjp(grad_out)
    _out0 = jnp.asarray(_out)
    return (_out0, *[jnp.asarray(_g) for _g in _grads])
```

```python
import functools
import math

import numpy as np
import jax
import jax.numpy as jnp
import jax.experimental.pallas as pl
import jax.experimental.pallas.tpu as pltpu

S = 2048
D = 576
DF = D // 2 + 1
DFP = 304
F = 4608
R1 = 16
R2 = 128
TF = 256
NF = F // TF
EPS = 1e-5

_NN = (((1,), (0,)), ((), ()))
_NT = (((1,), (1,)), ((), ()))
_TN = (((0,), (0,)), ((), ()))
_TT = (((0,), (1,)), ((), ()))


def _dg(a, b, dn):
    return jax.lax.dot_general(a, b, dn, preferred_element_type=jnp.float32)


def _const_tables():
    f = np.arange(DFP)[:, None].astype(np.float64)
    d = np.arange(D)[None, :].astype(np.float64)
    ang = 2.0 * np.pi * ((f * d) % D) / D
    valid = (np.arange(DFP) < DF)[:, None]
    fd = np.concatenate([np.where(valid, np.cos(ang), 0.0),
                         np.where(valid, -np.sin(ang), 0.0)], axis=0)
    a = np.arange(R2)[:, None].astype(np.float64)
    b = np.arange(R2)[None, :].astype(np.float64)
    ang = 2.0 * np.pi * ((a * b) % R2) / R2
    fr, fi = np.cos(ang), -np.sin(ang)
    mf = np.block([[fr, fi], [-fi, fr]])
    mi = np.block([[fr, -fi], [fi, fr]])
    k1 = np.arange(R1)[:, None].astype(np.float64)
    s2 = np.arange(R2)[None, :].astype(np.float64)
    ang = 2.0 * np.pi * ((k1 * s2) % S) / S
    tw = np.concatenate([np.cos(ang), -np.sin(ang)], axis=0)
    return (fd.astype(np.float32), mf.astype(np.float32), mi.astype(np.float32),
            tw.astype(np.float32))


def _cmul_const(z, n, k, inverse):
    re, im = z
    if k == 0:
        return z
    sgn = 1.0 if inverse else -1.0
    if 4 * k == n:
        return (-sgn * im, sgn * re) if inverse else (im, -re)
    c = math.cos(2.0 * math.pi * k / n)
    s = sgn * math.sin(2.0 * math.pi * k / n)
    if 8 * k == n:
        if inverse:
            return ((re - im) * c, (re + im) * c)
        return ((re + im) * c, (im - re) * c)
    if 8 * k == 3 * n:
        cc = -c
        if inverse:
            return (-(re + im) * cc, (re - im) * cc)
        return ((im - re) * cc, -(re + im) * cc)
    return (re * c - im * s, re * s + im * c)


def _fft_list(xs, inverse):
    n = len(xs)
    if n == 1:
        return xs
    e = _fft_list(xs[0::2], inverse)
    o = _fft_list(xs[1::2], inverse)
    out = [None] * n
    for k in range(n // 2):
        t = _cmul_const(o[k], n, k, inverse)
        out[k] = (e[k][0] + t[0], e[k][1] + t[1])
        out[k + n // 2] = (e[k][0] - t[0], e[k][1] - t[1])
    return out


def _kernel(xT_hbm, doT_hbm, wrT_hbm, wiT_hbm, wg_hbm, wu_hbm, wdT_hbm,
            fd_ref, fdT_ref, mf_ref, mi_ref, tw_ref,
            outT_hbm, dxT_hbm, dwrT_hbm, dwiT_hbm, dwg_hbm, dwu_hbm, dwdT_hbm,
            xT_ref, doT_ref, wT_ref, oT_ref, dxT_ref, dwT_ref, wbuf, obuf,
            n1T_s, r1_s, hT_s, n2T_s, r2_s, n2_s, do_s, outT_s, dn2T_s,
            pt_s, b_s, x_s, w_s, wtmp_s, tr_s,
            sem_in, sem_w, sem_o, sem_out):
    SL = 8
    w_hbms = (wg_hbm, wu_hbm, wdT_hbm)
    dw_hbms = (dwg_hbm, dwu_hbm, dwdT_hbm)

    def w_copy(j, slot, t):
        return pltpu.make_async_copy(
            w_hbms[t].at[:, pl.ds(pl.multiple_of(j * TF, TF), TF)],
            wbuf.at[slot, t], sem_w.at[slot, t])

    def o_copy(j, slot, t):
        return pltpu.make_async_copy(
            obuf.at[slot, t],
            dw_hbms[t].at[:, pl.ds(pl.multiple_of(j * TF, TF), TF)],
            sem_o.at[slot, t])

    cp_wr = pltpu.make_async_copy(wrT_hbm, wT_ref.at[0], sem_in.at[0])
    cp_wi = pltpu.make_async_copy(wiT_hbm, wT_ref.at[1], sem_in.at[1])
    cp_x = pltpu.make_async_copy(xT_hbm, xT_ref, sem_in.at[2])
    cp_do = pltpu.make_async_copy(doT_hbm, doT_ref, sem_in.at[3])
    cp_wr.start()
    cp_wi.start()
    cp_x.start()
    cp_do.start()
    for t in range(3):
        w_copy(0, 0, t).start()

    def fwd_transform(uT_bf16):
        pt_s[...] = _dg(fd_ref[...], uT_bf16, _NN)

        def body(i, carry):
            r0 = pl.multiple_of(i * SL, SL)
            xs = [(pt_s[pl.ds(r0, SL), s1 * R2:(s1 + 1) * R2],
                   pt_s[pl.ds(DFP + r0, SL), s1 * R2:(s1 + 1) * R2]) for s1 in range(R1)]
            ys = _fft_list(xs, False)
            for k1 in range(R1):
                re, im = ys[k1]
                if k1 == 0:
                    b_s[k1, pl.ds(r0, SL), 0:R2] = re
                    b_s[k1, pl.ds(r0, SL), R2:2 * R2] = im
                else:
                    c = tw_ref[k1:k1 + 1, :]
                    s = tw_ref[R1 + k1:R1 + k1 + 1, :]
                    b_s[k1, pl.ds(r0, SL), 0:R2] = re * c - im * s
                    b_s[k1, pl.ds(r0, SL), R2:2 * R2] = re * s + im * c
            return carry
        jax.lax.fori_loop(0, DFP // SL, body, 0)
        bb = b_s[...].astype(jnp.bfloat16).reshape(R1 * DFP, 2 * R2)
        return _dg(bb, mf_ref[...], _NN)

    def inv_transform(v_bf16):
        b_s[...] = _dg(v_bf16, mi_ref[...], _NN).reshape(R1, DFP, 2 * R2)

        def body(i, carry):
            r0 = pl.multiple_of(i * SL, SL)
            xs = []
            for k1 in range(R1):
                re = b_s[k1, pl.ds(r0, SL), 0:R2]
                im = b_s[k1, pl.ds(r0, SL), R2:2 * R2]
                if k1 == 0:
                    xs.append((re, im))
                else:
                    c = tw_ref[k1:k1 + 1, :]
                    s = tw_ref[R1 + k1:R1 + k1 + 1, :]
                    xs.append((re * c + im * s, im * c - re * s))
            zs = _fft_list(xs, True)
            for s1 in range(R1):
                pt_s[pl.ds(r0, SL), s1 * R2:(s1 + 1) * R2] = zs[s1][0]
                pt_s[pl.ds(DFP + r0, SL), s1 * R2:(s1 + 1) * R2] = zs[s1][1]
            return carry
        jax.lax.fori_loop(0, DFP // SL, body, 0)
        return _dg(fdT_ref[...], pt_s[...].astype(jnp.bfloat16), _NN)

    def freq_scale():
        frow = jax.lax.broadcasted_iota(jnp.int32, (DFP, R2), 0)
        scale = jnp.where((frow == 0) | (frow == DF - 1), 1.0, 2.0) * (1.0 / (S * D))
        return jnp.where(frow < DF, scale, 0.0).astype(jnp.float32)

    with jax.named_scope("wprep"):
        scale = freq_scale()
        tr_s[DF - 1:384, :] = jnp.zeros((384 - DF + 1, S), jnp.float32)
        for c, cp in enumerate((cp_wr, cp_wi)):
            cp.wait()
            tr_s[0:DF, :] = wT_ref[c].astype(jnp.float32)
            for q in range(3):
                wtmp_s[q] = tr_s[q * 128:(q + 1) * 128, :].T
            for k1 in range(R1):
                for q in range(3):
                    nr = min(128, DFP - q * 128)
                    blk = wtmp_s[q, pl.ds(k1, R2, stride=R1), :]
                    w_s[k1, q * 128:q * 128 + nr, c * R2:(c + 1) * R2] = (
                        blk.T[0:nr, :] * scale[q * 128:q * 128 + nr, :])

    with jax.named_scope("ln1"):
        cp_x.wait()
        x = xT_ref[...].astype(jnp.float32)
        m = jnp.mean(x, axis=0, keepdims=True)
        xc = x - m
        v = jnp.mean(xc * xc, axis=0, keepdims=True)
        r1 = jax.lax.rsqrt(v + EPS)
        n1T_s[...] = (xc * r1).astype(jnp.bfloat16)
        r1_s[...] = r1

    with jax.named_scope("fwd1"):
        x_s[...] = fwd_transform(n1T_s[...]).reshape(R1, DFP, 2 * R2)
    with jax.named_scope("mulw"):
        xr = x_s[:, :, 0:R2]
        xi = x_s[:, :, R2:2 * R2]
        wr = w_s[:, :, 0:R2]
        wi = w_s[:, :, R2:2 * R2]
        b_s[:, :, 0:R2] = xr * wr - xi * wi
        b_s[:, :, R2:2 * R2] = xr * wi + xi * wr
    with jax.named_scope("inv1"):
        y = inv_transform(b_s[...].astype(jnp.bfloat16).reshape(R1 * DFP, 2 * R2))
        hT_s[...] = xT_ref[...].astype(jnp.float32) + y

    with jax.named_scope("ln2"):
        h = hT_s[...]
        m = jnp.mean(h, axis=0, keepdims=True)
        hc = h - m
        v = jnp.mean(hc * hc, axis=0, keepdims=True)
        r2 = jax.lax.rsqrt(v + EPS)
        n2T = (hc * r2).astype(jnp.bfloat16)
        n2T_s[...] = n2T
        r2_s[...] = r2
        n2_s[...] = n2T.T
        cp_do.wait()
        do_s[...] = doT_ref[...].T
        outT_s[...] = jnp.zeros_like(outT_s)
        dn2T_s[...] = jnp.zeros_like(dn2T_s)

    def ffn_step(j, carry):
        slot = jax.lax.rem(j, 2)
        for t in range(3):
            w_copy(j, slot, t).wait()

        @pl.when(j + 1 < NF)
        def _():
            for t in range(3):
                w_copy(j + 1, 1 - slot, t).start()

        @pl.when(j >= 2)
        def _():
            for t in range(3):
                o_copy(j - 2, slot, t).wait()

        with jax.named_scope("ffn"):
            n2 = n2_s[...]
            wg = wbuf[slot, 0]
            wu = wbuf[slot, 1]
            wdT = wbuf[slot, 2]
            a = _dg(n2, wg, _NN)
            b = _dg(n2, wu, _NN)
            dgu = _dg(do_s[...], wdT, _NN)
            sig = jax.nn.sigmoid(a)
            g = a * sig
            gu = (g * b).astype(jnp.bfloat16)
            dgg = dgu * b
            db = (dgu * g).astype(jnp.bfloat16)
            da = (dgg * (sig * (1.0 + a * (1.0 - sig)))).astype(jnp.bfloat16)
            outT_s[...] += _dg(wdT, gu, _NT)
            dn2T_s[...] += _dg(wg, da, _NT) + _dg(wu, db, _NT)
            obuf[slot, 2] = _dg(doT_ref[...], gu, _NN).astype(jnp.bfloat16)
            obuf[slot, 0] = _dg(n2T_s[...], da, _NN).astype(jnp.bfloat16)
            obuf[slot, 1] = _dg(n2T_s[...], db, _NN).astype(jnp.bfloat16)
        for t in range(3):
            o_copy(j, slot, t).start()
        return carry

    jax.lax.fori_loop(0, NF, ffn_step, 0)

    cp_out = pltpu.make_async_copy(oT_ref, outT_hbm, sem_out.at[0])
    cp_dx = pltpu.make_async_copy(dxT_ref, dxT_hbm, sem_out.at[1])
    cp_dwr = pltpu.make_async_copy(dwT_ref.at[0], dwrT_hbm, sem_out.at[2])
    cp_dwi = pltpu.make_async_copy(dwT_ref.at[1], dwiT_hbm, sem_out.at[3])
    with jax.named_scope("ln2b"):
        oT_ref[...] = (hT_s[...] + outT_s[...]).astype(jnp.bfloat16)
        cp_out.start()
        dn2 = dn2T_s[...]
        n2f = n2T_s[...].astype(jnp.float32)
        c1 = jnp.mean(dn2, axis=0, keepdims=True)
        c2 = jnp.mean(dn2 * n2f, axis=0, keepdims=True)
        dh = doT_ref[...].astype(jnp.float32) + r2_s[...] * (dn2 - c1 - n2f * c2)
        hT_s[...] = dh

    with jax.named_scope("fwd2"):
        G = fwd_transform(hT_s[...].astype(jnp.bfloat16)).reshape(R1, DFP, 2 * R2)
    with jax.named_scope("mulw2"):
        gr = G[:, :, 0:R2]
        gi = G[:, :, R2:2 * R2]
        xr = x_s[:, :, 0:R2]
        xi = x_s[:, :, R2:2 * R2]
        scale = freq_scale()
        x_s[:, :, 0:R2] = (gr * xr + gi * xi) * scale
        x_s[:, :, R2:2 * R2] = (gi * xr - gr * xi) * scale
        wr = w_s[:, :, 0:R2]
        wi = w_s[:, :, R2:2 * R2]
        b_s[:, :, 0:R2] = gr * wr + gi * wi
        b_s[:, :, R2:2 * R2] = gi * wr - gr * wi

    with jax.named_scope("dwout"):
        zpad = jnp.zeros((128 - (DFP - 256), R2), jnp.float32)
        for c, cp in enumerate((cp_dwr, cp_dwi)):
            for k1 in range(R1):
                for q in range(3):
                    if q < 2:
                        blk = x_s[k1, q * 128:(q + 1) * 128, c * R2:(c + 1) * R2]
                    else:
                        blk = jnp.concatenate(
                            [x_s[k1, 256:DFP, c * R2:(c + 1) * R2], zpad], axis=0)
                    wtmp_s[q, pl.ds(k1, R2, stride=R1), :] = blk.T
            for q in range(3):
                tr_s[q * 128:(q + 1) * 128, :] = wtmp_s[q].T
            dwT_ref[c] = tr_s[0:DF, :].astype(jnp.bfloat16)
            cp.start()

    with jax.named_scope("inv2"):
        dn1 = inv_transform(b_s[...].astype(jnp.bfloat16).reshape(R1 * DFP, 2 * R2))
    with jax.named_scope("ln1b"):
        n1f = n1T_s[...].astype(jnp.float32)
        c1 = jnp.mean(dn1, axis=0, keepdims=True)
        c2 = jnp.mean(dn1 * n1f, axis=0, keepdims=True)
        dxT_ref[...] = (hT_s[...] + r1_s[...] * (dn1 - c1 - n1f * c2)).astype(jnp.bfloat16)
    cp_dx.start()

    for jj in (NF - 2, NF - 1):
        for t in range(3):
            o_copy(jj, jj % 2, t).wait()
    cp_out.wait()
    cp_dwr.wait()
    cp_dwi.wait()
    cp_dx.wait()


@jax.jit
def pallas_sequential_preLN__spectral_gfnet__swiglu_ffn__prompt_kernel(
    A_x: jax.Array,
    A_w_r: jax.Array,
    A_w_i: jax.Array,
    B_x: jax.Array,
    B_w_gate: jax.Array,
    B_w_up: jax.Array,
    B_w_down: jax.Array,
    grad_out: jax.Array,
):
    xT = A_x.reshape(S, D).T
    doT = grad_out.reshape(S, D).T
    wrT = A_w_r.T
    wiT = A_w_i.T
    wdT = B_w_down.T
    fd, mf, mi, tw = _const_tables()
    fdT = jnp.asarray(np.ascontiguousarray(fd.T), dtype=jnp.bfloat16)
    fd = jnp.asarray(fd, dtype=jnp.bfloat16)
    mf = jnp.asarray(mf, dtype=jnp.bfloat16)
    mi = jnp.asarray(mi, dtype=jnp.bfloat16)
    tw = jnp.asarray(tw, dtype=jnp.float32)

    hbm = pl.BlockSpec(memory_space=pl.ANY)
    vmem = pl.BlockSpec(memory_space=pltpu.VMEM)
    in_specs = [hbm] * 7 + [vmem] * 5
    out_specs = [hbm] * 7
    bf = jnp.bfloat16
    out_shape = [
        jax.ShapeDtypeStruct((D, S), bf), jax.ShapeDtypeStruct((D, S), bf),
        jax.ShapeDtypeStruct((DF, S), bf), jax.ShapeDtypeStruct((DF, S), bf),
        jax.ShapeDtypeStruct((D, F), bf), jax.ShapeDtypeStruct((D, F), bf),
        jax.ShapeDtypeStruct((D, F), bf),
    ]
    f32 = jnp.float32
    scratch = [
        pltpu.VMEM((D, S), bf),
        pltpu.VMEM((D, S), bf),
        pltpu.VMEM((2, DF, S), bf),
        pltpu.VMEM((D, S), bf),
        pltpu.VMEM((D, S), bf),
        pltpu.VMEM((2, DF, S), bf),
        pltpu.VMEM((2, 3, D, TF), bf),
        pltpu.VMEM((2, 3, D, TF), bf),
        pltpu.VMEM((D, S), bf),
        pltpu.VMEM((1, S), f32),
        pltpu.VMEM((D, S), f32),
        pltpu.VMEM((D, S), bf),
        pltpu.VMEM((1, S), f32),
        pltpu.VMEM((S, D), bf),
        pltpu.VMEM((S, D), bf),
        pltpu.VMEM((D, S), f32),
        pltpu.VMEM((D, S), f32),
        pltpu.VMEM((2 * DFP, S), f32),
        pltpu.VMEM((R1, DFP, 2 * R2), f32),
        pltpu.VMEM((R1, DFP, 2 * R2), f32),
        pltpu.VMEM((R1, DFP, 2 * R2), f32),
        pltpu.VMEM((3, S, 128), f32),
        pltpu.VMEM((384, S), f32),
        pltpu.SemaphoreType.DMA((4,)),
        pltpu.SemaphoreType.DMA((2, 3)),
        pltpu.SemaphoreType.DMA((2, 3)),
        pltpu.SemaphoreType.DMA((4,)),
    ]
    outs = pl.pallas_call(
        _kernel,
        in_specs=in_specs,
        out_specs=out_specs,
        out_shape=out_shape,
        scratch_shapes=scratch,
        compiler_params=pltpu.CompilerParams(
            vmem_limit_bytes=120 * 1024 * 1024,
        ),
    )(xT, doT, wrT, wiT, B_w_gate, B_w_up, wdT, fd, fdT, mf, mi, tw)
    outT, dxT, dwrT, dwiT, dwg, dwu, dwdT = outs
    return (outT.T.reshape(1, S, D), dxT.T.reshape(1, S, D), dwrT.T, dwiT.T, dwg, dwu, dwdT.T)
```

```python
import contextlib
import math

import numpy as np
import jax
import jax.numpy as jnp
import jax.experimental.pallas as pl
import jax.experimental.pallas.tpu as pltpu

S = 2048
D = 576
H = D // 2
DF = D // 2 + 1
NE = 160
NO = 144
DFP = NE + NO
F = 4608
R1 = 16
R2 = 128
TF = 128
NF = F // TF
EPS = 1e-5
SLB = 16
_SLABS = ([(r, min(SLB, NE - r)) for r in range(0, NE, SLB)]
          + [(r, min(SLB, DFP - r)) for r in range(NE, DFP, SLB)])
NC = 4
CW = S // NC
NC2 = 4
CW2 = S // NC2

_NN = (((1,), (0,)), ((), ()))
_NT = (((1,), (1,)), ((), ()))

_FINE_SCOPES = ("ffn",)


def _scope(name):
    return jax.named_scope(name) if name in _FINE_SCOPES else contextlib.nullcontext()


def _dg(a, b, dn):
    return jax.lax.dot_general(a, b, dn, preferred_element_type=jnp.float32)


def _const_tables():
    d = np.arange(H)[None, :].astype(np.float64)
    f2 = np.arange(NE)[:, None].astype(np.float64)
    ang = 2.0 * np.pi * ((f2 * d) % H) / H
    valid = (np.arange(NE) <= H // 2)[:, None]
    fe = np.concatenate([np.where(valid, np.cos(ang), 0.0),
                         np.where(valid, -np.sin(ang), 0.0)], axis=0)
    f2 = np.arange(NO)[:, None].astype(np.float64)
    ang = 2.0 * np.pi * (((2 * f2 + 1) * d) % D) / D
    fo = np.concatenate([np.cos(ang), -np.sin(ang)], axis=0)
    a = np.arange(R2)[:, None].astype(np.float64)
    b = np.arange(R2)[None, :].astype(np.float64)
    ang = 2.0 * np.pi * ((a * b) % R2) / R2
    fr, fi = np.cos(ang), -np.sin(ang)
    mf = np.block([[fr, fi], [-fi, fr]])
    mi = np.block([[fr, -fi], [fi, fr]])
    k1 = np.arange(R1)[:, None].astype(np.float64)
    s2 = np.arange(R2)[None, :].astype(np.float64)
    ang = 2.0 * np.pi * ((k1 * s2) % S) / S
    tw = np.concatenate([np.cos(ang), -np.sin(ang)], axis=0)
    return fe, fo, mf, mi, tw


def _cmul_const(z, n, k, inverse):
    re, im = z
    if k == 0:
        return z
    sgn = 1.0 if inverse else -1.0
    if 4 * k == n:
        return (-im, re) if inverse else (im, -re)
    c = math.cos(2.0 * math.pi * k / n)
    s = sgn * math.sin(2.0 * math.pi * k / n)
    if 8 * k == n:
        if inverse:
            return ((re - im) * c, (re + im) * c)
        return ((re + im) * c, (im - re) * c)
    if 8 * k == 3 * n:
        cc = -c
        if inverse:
            return (-(re + im) * cc, (re - im) * cc)
        return ((im - re) * cc, -(re + im) * cc)
    return (re * c - im * s, re * s + im * c)


def _fft_list(xs, inverse):
    n = len(xs)
    if n == 1:
        return xs
    e = _fft_list(xs[0::2], inverse)
    o = _fft_list(xs[1::2], inverse)
    out = [None] * n
    for k in range(n // 2):
        t = _cmul_const(o[k], n, k, inverse)
        out[k] = (e[k][0] + t[0], e[k][1] + t[1])
        out[k + n // 2] = (e[k][0] - t[0], e[k][1] - t[1])
    return out


def _rows(r0):
    if r0 < NE:
        return r0, NE + r0
    return 2 * NE + (r0 - NE), 2 * NE + NO + (r0 - NE)


def _kernel(xT_hbm, doT_hbm, wrT_hbm, wiT_hbm, wg_hbm, wu_hbm, wdT_hbm,
            fe_hbm, fo_hbm, ge_hbm, go_hbm, mf_hbm, mi_hbm, tw_hbm,
            outT_hbm, dxT_hbm, dwrT_hbm, dwiT_hbm, dwg_hbm, dwu_hbm, dwdT_hbm,
            fe_ref, fo_ref, ge_ref, go_ref, mf_ref, mi_ref, tw_ref,
            xT_ref, doT_ref, wT_ref, oT_ref, dxT_ref, dwT_ref, wbuf, obuf,
            n1T_s, r1_s, hT_s, n2T_s, r2_s, n2_s, do_s, outT_s, dn2T_s,
            a_s, pt_s, zt_s, x_s, w_s, wtmp_s, tr_s,
            sem_x, sem_in, sem_c, sem_w, sem_o, sem_dx, sem_out):
    f32 = jnp.float32
    bf16 = jnp.bfloat16
    w_hbms = (wg_hbm, wu_hbm, wdT_hbm)
    dw_hbms = (dwg_hbm, dwu_hbm, dwdT_hbm)

    def w_copy(j, slot, t):
        return pltpu.make_async_copy(
            w_hbms[t].at[:, pl.ds(pl.multiple_of(j * TF, TF), TF)],
            wbuf.at[slot, t], sem_w.at[slot, t])

    def o_copy(j, slot, t):
        return pltpu.make_async_copy(
            obuf.at[slot, t],
            dw_hbms[t].at[:, pl.ds(pl.multiple_of(j * TF, TF), TF)],
            sem_o.at[slot, t])

    cp_x = [pltpu.make_async_copy(xT_hbm.at[:, c * CW:(c + 1) * CW],
                                  xT_ref.at[:, c * CW:(c + 1) * CW], sem_x.at[c])
            for c in range(NC)]
    cp_c = [pltpu.make_async_copy(src, dst, sem_c.at[i]) for i, (src, dst) in enumerate(
        ((fe_hbm, fe_ref), (fo_hbm, fo_ref), (mf_hbm, mf_ref), (mi_hbm, mi_ref),
         (tw_hbm, tw_ref), (ge_hbm, ge_ref), (go_hbm, go_ref)))]
    cp_wr = pltpu.make_async_copy(wrT_hbm, wT_ref.at[0], sem_in.at[0])
    cp_wi = pltpu.make_async_copy(wiT_hbm, wT_ref.at[1], sem_in.at[1])
    cp_do = pltpu.make_async_copy(doT_hbm, doT_ref, sem_in.at[2])

    cp_x[0].start()
    cp_c[0].start()
    cp_c[1].start()
    tr_s[NO:256, :] = jnp.zeros((256 - NO, S), jnp.uint32)

    def fwd_a(cs):
        pt_s[0:2 * NE, cs] = _dg(fe_ref[...], a_s[0:H, cs], _NN)
        pt_s[2 * NE:2 * DFP, cs] = _dg(fo_ref[...], a_s[H:D, cs], _NN)

    def split_store(u, cs):
        a_s[0:H, cs] = (u[0:H] + u[H:D]).astype(bf16)
        a_s[H:D, cs] = (u[0:H] - u[H:D]).astype(bf16)

    def inv_b(cs):
        e = _dg(ge_ref[...], zt_s[0:2 * NE, cs], _NN)
        o = _dg(go_ref[...], zt_s[2 * NE:2 * DFP, cs], _NN)
        return jnp.concatenate([e + o, e - o], axis=0)

    def middle(pointwise):
        for r0, sl in _SLABS:
            rs = slice(r0, r0 + sl)
            rre, rim = _rows(r0)
            xs = [(pt_s[rre:rre + sl, s1 * R2:(s1 + 1) * R2],
                   pt_s[rim:rim + sl, s1 * R2:(s1 + 1) * R2]) for s1 in range(R1)]
            ys = _fft_list(xs, False)
            rows = []
            for k1 in range(R1):
                re, im = ys[k1]
                if k1 > 0:
                    c = tw_ref[k1:k1 + 1, :]
                    sn = tw_ref[R1 + k1:R1 + k1 + 1, :]
                    re, im = re * c - im * sn, re * sn + im * c
                rows.append(jnp.concatenate([re, im], axis=1))
            bb = jnp.concatenate(rows, axis=0).astype(bf16)
            X = _dg(bb, mf_ref[...], _NN).reshape(R1, sl, 2 * R2)
            V = pointwise(X, rs)
            C = _dg(V.reshape(R1 * sl, 2 * R2).astype(bf16), mi_ref[...], _NN)
            C = C.reshape(R1, sl, 2 * R2)
            xs = []
            for k1 in range(R1):
                re = C[k1, :, 0:R2]
                im = C[k1, :, R2:2 * R2]
                if k1 > 0:
                    c = tw_ref[k1:k1 + 1, :]
                    sn = tw_ref[R1 + k1:R1 + k1 + 1, :]
                    re, im = re * c + im * sn, im * c - re * sn
                xs.append((re, im))
            zs = _fft_list(xs, True)
            for s1 in range(R1):
                zt_s[rre:rre + sl, s1 * R2:(s1 + 1) * R2] = zs[s1][0].astype(bf16)
                zt_s[rim:rim + sl, s1 * R2:(s1 + 1) * R2] = zs[s1][1].astype(bf16)

    def freq_scale():
        r = jax.lax.broadcasted_iota(jnp.int32, (DFP, R2), 0)
        scale = jnp.where((r == 0) | (r == H // 2), 1.0, 2.0) * (1.0 / (S * D))
        return jnp.where((r <= H // 2) | (r >= NE), scale, 0.0).astype(f32)

    def ln1_chunk(c):
        cs = slice(c * CW, (c + 1) * CW)
        x = xT_ref[:, cs].astype(f32)
        m = jnp.mean(x, axis=0, keepdims=True)
        xc = x - m
        v = jnp.mean(xc * xc, axis=0, keepdims=True)
        r1 = jax.lax.rsqrt(v + EPS)
        n1 = xc * r1
        n1T_s[:, cs] = n1.astype(bf16)
        r1_s[:, cs] = r1
        split_store(n1, cs)
        fwd_a(cs)

    def wprep(c):
        scale = freq_scale()
        hi = jnp.uint32(0xFFFF0000)
        tr_s[0:NO, :] = pltpu.bitcast(wT_ref[c, 0:H, :], jnp.uint32)
        tr_s[NO:NO + 1, :] = pltpu.bitcast(wT_ref[c, H:DF, :].astype(f32), jnp.uint32) >> 16
        for q in range(2):
            wtmp_s[q] = tr_s[q * 128:(q + 1) * 128, :].T
        for k1 in range(R1):
            b0 = wtmp_s[0, pl.ds(k1, R2, stride=R1), :].T
            b1 = wtmp_s[1, pl.ds(k1, R2, stride=R1), :].T[0:NE - 128, :]
            u = jnp.concatenate([b0, b1], axis=0)
            cl = slice(c * R2, (c + 1) * R2)
            w_s[k1, 0:NE, cl] = pltpu.bitcast(u << 16, f32) * scale[0:NE]
            w_s[k1, NE:DFP, cl] = pltpu.bitcast(u[0:NO] & hi, f32) * scale[NE:DFP]

    with _scope("ln1"):
        cp_x[0].wait()
        cp_c[0].wait()
        cp_c[1].wait()
        cp_wr.start()
        cp_x[1].start()
        ln1_chunk(0)
        cp_wr.wait()
        cp_x[1].wait()
        cp_wi.start()
        cp_x[2].start()
        wprep(0)
        ln1_chunk(1)
        cp_wi.wait()
        cp_x[2].wait()
        cp_x[3].start()
        for i in range(2, 5):
            cp_c[i].start()
        wprep(1)
        ln1_chunk(2)
        cp_x[3].wait()
        for i in range(5, 7):
            cp_c[i].start()
        cp_do.start()
        for t in range(3):
            w_copy(0, 0, t).start()
        ln1_chunk(3)
        for i in range(2, 5):
            cp_c[i].wait()

    def pw_fwd(X, rs):
        x_s[:, rs, :] = X
        xr = X[:, :, 0:R2]
        xi = X[:, :, R2:2 * R2]
        wr = w_s[:, rs, 0:R2]
        wi = w_s[:, rs, R2:2 * R2]
        return jnp.concatenate([xr * wr - xi * wi, xr * wi + xi * wr], axis=2)

    with _scope("mid1"):
        middle(pw_fwd)

    with _scope("ln2"):
        cp_c[5].wait()
        cp_c[6].wait()
        cp_do.wait()
        do_s[...] = doT_ref[...].T
        for c in range(NC2):
            cs = slice(c * CW2, (c + 1) * CW2)
            h = xT_ref[:, cs].astype(f32) + inv_b(cs)
            outT_s[:, cs] = h
            m = jnp.mean(h, axis=0, keepdims=True)
            hc = h - m
            v = jnp.mean(hc * hc, axis=0, keepdims=True)
            r2 = jax.lax.rsqrt(v + EPS)
            n2T = (hc * r2).astype(bf16)
            n2T_s[:, cs] = n2T
            r2_s[:, cs] = r2
            n2_s[cs, :] = n2T.T
        dn2T_s[...] = jnp.zeros_like(dn2T_s)

    def ffn_step(j, carry):
        slot = jax.lax.rem(j, 2)
        for t in range(3):
            w_copy(j, slot, t).wait()

        @pl.when(j + 1 < NF)
        def _():
            for t in range(3):
                w_copy(j + 1, 1 - slot, t).start()

        @pl.when(j >= 2)
        def _():
            for t in range(3):
                o_copy(j - 2, slot, t).wait()

        with _scope("ffn"):
            n2 = n2_s[...]
            wg = wbuf[slot, 0]
            wu = wbuf[slot, 1]
            wdT = wbuf[slot, 2]
            a = _dg(n2, wg, _NN)
            b = _dg(n2, wu, _NN)
            dgu = _dg(do_s[...], wdT, _NN)
            sig = jax.nn.sigmoid(a)
            g = a * sig
            gu = (g * b).astype(bf16)
            dgg = dgu * b
            db = (dgu * g).astype(bf16)
            da = (dgg * (sig * (1.0 + a * (1.0 - sig)))).astype(bf16)
            outT_s[...] += _dg(wdT, gu, _NT)
            dn2T_s[...] += _dg(wg, da, _NT) + _dg(wu, db, _NT)
            obuf[slot, 2] = _dg(doT_ref[...], gu, _NN).astype(bf16)
            obuf[slot, 0] = _dg(n2T_s[...], da, _NN).astype(bf16)
            obuf[slot, 1] = _dg(n2T_s[...], db, _NN).astype(bf16)
        for t in range(3):
            o_copy(j, slot, t).start()
        return carry

    jax.lax.fori_loop(0, NF, ffn_step, 0)

    cp_out = pltpu.make_async_copy(oT_ref, outT_hbm, sem_out.at[0])
    cp_dwr = pltpu.make_async_copy(dwT_ref.at[0], dwrT_hbm, sem_out.at[1])
    cp_dwi = pltpu.make_async_copy(dwT_ref.at[1], dwiT_hbm, sem_out.at[2])
    cp_dx = [pltpu.make_async_copy(dxT_ref.at[:, c * CW2:(c + 1) * CW2],
                                   dxT_hbm.at[:, c * CW2:(c + 1) * CW2], sem_dx.at[c])
             for c in range(NC2)]
    with _scope("ln2b"):
        for c in range(NC2):
            cs = slice(c * CW2, (c + 1) * CW2)
            dn2 = dn2T_s[:, cs]
            n2f = n2T_s[:, cs].astype(f32)
            c1 = jnp.mean(dn2, axis=0, keepdims=True)
            c2 = jnp.mean(dn2 * n2f, axis=0, keepdims=True)
            dh = doT_ref[:, cs].astype(f32) + r2_s[:, cs] * (dn2 - c1 - n2f * c2)
            oT_ref[:, cs] = outT_s[:, cs].astype(bf16)
            hT_s[:, cs] = dh
            split_store(dh, cs)
            fwd_a(cs)
        cp_out.start()

    scale = freq_scale()

    def pw_bwd(G, rs):
        gr = G[:, :, 0:R2]
        gi = G[:, :, R2:2 * R2]
        xr = x_s[:, rs, 0:R2]
        xi = x_s[:, rs, R2:2 * R2]
        sc = scale[rs, :]
        x_s[:, rs, 0:R2] = (gr * xr + gi * xi) * sc
        x_s[:, rs, R2:2 * R2] = (gi * xr - gr * xi) * sc
        wr = w_s[:, rs, 0:R2]
        wi = w_s[:, rs, R2:2 * R2]
        return jnp.concatenate([gr * wr + gi * wi, gi * wr - gr * wi], axis=2)

    with _scope("mid2"):
        middle(pw_bwd)

    with _scope("tail"):
        hi = jnp.uint32(0xFFFF0000)
        zpad = jnp.zeros((256 - NE, R2), jnp.uint32)
        zodd = jnp.zeros((NE - NO, R2), jnp.uint32)
        for c in range(2):
            cl = slice(c * R2, (c + 1) * R2)
            for k1 in range(R1):
                ev = x_s[k1, 0:NE, cl].astype(bf16).astype(f32)
                od = x_s[k1, NE:DFP, cl].astype(bf16).astype(f32)
                u = (pltpu.bitcast(ev, jnp.uint32) >> 16) | jnp.concatenate(
                    [pltpu.bitcast(od, jnp.uint32) & hi, zodd], axis=0)
                wtmp_s[0, pl.ds(k1, R2, stride=R1), :] = u[0:128].T
                wtmp_s[1, pl.ds(k1, R2, stride=R1), :] = jnp.concatenate(
                    [u[128:NE], zpad], axis=0).T
            for q in range(2):
                tr_s[q * 128:(q + 1) * 128, :] = wtmp_s[q].T
            dwT_ref[c, 0:H, :] = pltpu.bitcast(tr_s[0:NO, :], bf16)
            dwT_ref[c, H:DF, :] = pltpu.bitcast(tr_s[NO:NO + 1, :] << 16, f32).astype(bf16)
            (cp_dwr, cp_dwi)[c].start()
        for c in range(NC2):
            cs = slice(c * CW2, (c + 1) * CW2)
            dn1 = inv_b(cs)
            n1f = n1T_s[:, cs].astype(f32)
            c1 = jnp.mean(dn1, axis=0, keepdims=True)
            c2 = jnp.mean(dn1 * n1f, axis=0, keepdims=True)
            dxT_ref[:, cs] = (hT_s[:, cs] + r1_s[:, cs] * (dn1 - c1 - n1f * c2)).astype(bf16)
            cp_dx[c].start()

    for jj in (NF - 2, NF - 1):
        for t in range(3):
            o_copy(jj, jj % 2, t).wait()
    cp_out.wait()
    cp_dwr.wait()
    cp_dwi.wait()
    for c in range(NC2):
        cp_dx[c].wait()


@jax.jit
def pallas_sequential_preLN__spectral_gfnet__swiglu_ffn__prompt_kernel(
    A_x: jax.Array,
    A_w_r: jax.Array,
    A_w_i: jax.Array,
    B_x: jax.Array,
    B_w_gate: jax.Array,
    B_w_up: jax.Array,
    B_w_down: jax.Array,
    grad_out: jax.Array,
):
    xT = A_x.reshape(S, D).T
    doT = grad_out.reshape(S, D).T
    wrT = A_w_r.T
    wiT = A_w_i.T
    wdT = B_w_down.T
    bf = jnp.bfloat16
    f32 = jnp.float32
    fe, fo, mf, mi, tw = _const_tables()
    consts = [
        jnp.asarray(fe, dtype=bf), jnp.asarray(fo, dtype=bf),
        jnp.asarray(np.ascontiguousarray(fe.T), dtype=bf),
        jnp.asarray(np.ascontiguousarray(fo.T), dtype=bf),
        jnp.asarray(mf, dtype=bf), jnp.asarray(mi, dtype=bf),
        jnp.asarray(tw, dtype=f32),
    ]

    hbm = pl.BlockSpec(memory_space=pl.ANY)
    in_specs = [hbm] * 14
    out_specs = [hbm] * 7
    out_shape = [
        jax.ShapeDtypeStruct((D, S), bf), jax.ShapeDtypeStruct((D, S), bf),
        jax.ShapeDtypeStruct((DF, S), bf), jax.ShapeDtypeStruct((DF, S), bf),
        jax.ShapeDtypeStruct((D, F), bf), jax.ShapeDtypeStruct((D, F), bf),
        jax.ShapeDtypeStruct((D, F), bf),
    ]
    scratch = [pltpu.VMEM(c.shape, c.dtype) for c in consts] + [
        pltpu.VMEM((D, S), bf),
        pltpu.VMEM((D, S), bf),
        pltpu.VMEM((2, DF, S), bf),
        pltpu.VMEM((D, S), bf),
        pltpu.VMEM((D, S), bf),
        pltpu.VMEM((2, DF, S), bf),
        pltpu.VMEM((2, 3, D, TF), bf),
        pltpu.VMEM((2, 3, D, TF), bf),
        pltpu.VMEM((D, S), bf),
        pltpu.VMEM((1, S), f32),
        pltpu.VMEM((D, S), f32),
        pltpu.VMEM((D, S), bf),
        pltpu.VMEM((1, S), f32),
        pltpu.VMEM((S, D), bf),
        pltpu.VMEM((S, D), bf),
        pltpu.VMEM((D, S), f32),
        pltpu.VMEM((D, S), f32),
        pltpu.VMEM((D, S), bf),
        pltpu.VMEM((2 * DFP, S), f32),
        pltpu.VMEM((2 * DFP, S), bf),
        pltpu.VMEM((R1, DFP, 2 * R2), f32),
        pltpu.VMEM((R1, DFP, 2 * R2), f32),
        pltpu.VMEM((2, S, 128), jnp.uint32),
        pltpu.VMEM((256, S), jnp.uint32),
        pltpu.SemaphoreType.DMA((NC,)),
        pltpu.SemaphoreType.DMA((3,)),
        pltpu.SemaphoreType.DMA((7,)),
        pltpu.SemaphoreType.DMA((2, 3)),
        pltpu.SemaphoreType.DMA((2, 3)),
        pltpu.SemaphoreType.DMA((NC2,)),
        pltpu.SemaphoreType.DMA((3,)),
    ]
    outs = pl.pallas_call(
        _kernel,
        in_specs=in_specs,
        out_specs=out_specs,
        out_shape=out_shape,
        scratch_shapes=scratch,
        compiler_params=pltpu.CompilerParams(
            vmem_limit_bytes=120 * 1024 * 1024,
        ),
    )(xT, doT, wrT, wiT, B_w_gate, B_w_up, wdT, *consts)
    outT, dxT, dwrT, dwiT, dwg, dwu, dwdT = outs
    return (outT.T.reshape(1, S, D), dxT.T.reshape(1, S, D), dwrT.T, dwiT.T, dwg, dwu, dwdT.T)
```

```python
import contextlib
import math

import numpy as np
import jax
import jax.numpy as jnp
import jax.experimental.pallas as pl
import jax.experimental.pallas.tpu as pltpu

S = 2048
D = 576
H = D // 2
DF = D // 2 + 1
NE = 160
NO = 144
DFP = NE + NO
F = 4608
R1 = 16
R2 = 128
TF = 128
NF = F // TF
EPS = 1e-5
SLB = 16
_SLABS = ([(r, min(SLB, NE - r)) for r in range(0, NE, SLB)]
          + [(r, min(SLB, DFP - r)) for r in range(NE, DFP, SLB)])
LEAD_SLABS = 8
NC = 4
CW = S // NC
NC2 = 4
CW2 = S // NC2

_NN = (((1,), (0,)), ((), ()))
_NT = (((1,), (1,)), ((), ()))

_FINE_SCOPES = ("ffn",)


def _scope(name):
    return jax.named_scope(name) if name in _FINE_SCOPES else contextlib.nullcontext()


def _dg(a, b, dn):
    return jax.lax.dot_general(a, b, dn, preferred_element_type=jnp.float32)


def _const_tables():
    d = np.arange(H)[None, :].astype(np.float64)
    f2 = np.arange(NE)[:, None].astype(np.float64)
    ang = 2.0 * np.pi * ((f2 * d) % H) / H
    valid = (np.arange(NE) <= H // 2)[:, None]
    fe = np.concatenate([np.where(valid, np.cos(ang), 0.0),
                         np.where(valid, -np.sin(ang), 0.0)], axis=0)
    f2 = np.arange(NO)[:, None].astype(np.float64)
    ang = 2.0 * np.pi * (((2 * f2 + 1) * d) % D) / D
    fo = np.concatenate([np.cos(ang), -np.sin(ang)], axis=0)
    a = np.arange(R2)[:, None].astype(np.float64)
    b = np.arange(R2)[None, :].astype(np.float64)
    ang = 2.0 * np.pi * ((a * b) % R2) / R2
    fr, fi = np.cos(ang), -np.sin(ang)
    mf = np.block([[fr, fi], [-fi, fr]])
    mi = np.block([[fr, -fi], [fi, fr]])
    k1 = np.arange(R1)[:, None].astype(np.float64)
    s2 = np.arange(R2)[None, :].astype(np.float64)
    ang = 2.0 * np.pi * ((k1 * s2) % S) / S
    tw = np.concatenate([np.cos(ang), -np.sin(ang)], axis=0)
    return fe, fo, mf, mi, tw


def _cmul_const(z, n, k, inverse):
    re, im = z
    if k == 0:
        return z
    sgn = 1.0 if inverse else -1.0
    if 4 * k == n:
        return (-im, re) if inverse else (im, -re)
    c = math.cos(2.0 * math.pi * k / n)
    s = sgn * math.sin(2.0 * math.pi * k / n)
    if 8 * k == n:
        if inverse:
            return ((re - im) * c, (re + im) * c)
        return ((re + im) * c, (im - re) * c)
    if 8 * k == 3 * n:
        cc = -c
        if inverse:
            return (-(re + im) * cc, (re - im) * cc)
        return ((im - re) * cc, -(re + im) * cc)
    return (re * c - im * s, re * s + im * c)


def _fft_list(xs, inverse):
    n = len(xs)
    if n == 1:
        return xs
    e = _fft_list(xs[0::2], inverse)
    o = _fft_list(xs[1::2], inverse)
    out = [None] * n
    for k in range(n // 2):
        t = _cmul_const(o[k], n, k, inverse)
        out[k] = (e[k][0] + t[0], e[k][1] + t[1])
        out[k + n // 2] = (e[k][0] - t[0], e[k][1] - t[1])
    return out


def _rows(r0):
    if r0 < NE:
        return r0, NE + r0
    return 2 * NE + (r0 - NE), 2 * NE + NO + (r0 - NE)


def _kernel(xT_hbm, doT_hbm, wrT_hbm, wiT_hbm, wg_hbm, wu_hbm, wdT_hbm,
            fe_hbm, fo_hbm, ge_hbm, go_hbm, mf_hbm, mi_hbm, tw_hbm,
            outT_hbm, dxT_hbm, dwrT_hbm, dwiT_hbm, dwg_hbm, dwu_hbm, dwdT_hbm,
            fe_ref, fo_ref, ge_ref, go_ref, mf_ref, mi_ref, tw_ref,
            xT_ref, doT_ref, wT_ref, oT_ref, dxT_ref, dwT_ref, wbuf, obuf,
            n1T_s, r1_s, hT_s, n2T_s, r2_s, n2_s, do_s, outT_s, dn2T_s,
            a_s, pt_s, zt_s, x_s, w_s, wtmp_s, tr_s,
            sem_x, sem_in, sem_c, sem_w, sem_o, sem_dx, sem_out):
    f32 = jnp.float32
    bf16 = jnp.bfloat16
    w_hbms = (wg_hbm, wu_hbm, wdT_hbm)
    dw_hbms = (dwg_hbm, dwu_hbm, dwdT_hbm)

    def w_copy(j, slot, t):
        return pltpu.make_async_copy(
            w_hbms[t].at[:, pl.ds(pl.multiple_of(j * TF, TF), TF)],
            wbuf.at[slot, t], sem_w.at[slot, t])

    def o_copy(j, slot, t):
        return pltpu.make_async_copy(
            obuf.at[slot, t],
            dw_hbms[t].at[:, pl.ds(pl.multiple_of(j * TF, TF), TF)],
            sem_o.at[slot, t])

    cp_x = [pltpu.make_async_copy(xT_hbm.at[:, c * CW:(c + 1) * CW],
                                  xT_ref.at[:, c * CW:(c + 1) * CW], sem_x.at[c])
            for c in range(NC)]
    cp_c = [pltpu.make_async_copy(src, dst, sem_c.at[i]) for i, (src, dst) in enumerate(
        ((fe_hbm, fe_ref), (fo_hbm, fo_ref), (mf_hbm, mf_ref), (mi_hbm, mi_ref),
         (tw_hbm, tw_ref), (ge_hbm, ge_ref), (go_hbm, go_ref)))]
    cp_wr = pltpu.make_async_copy(wrT_hbm, wT_ref.at[0], sem_in.at[0])
    cp_wi = pltpu.make_async_copy(wiT_hbm, wT_ref.at[1], sem_in.at[1])
    cp_do = pltpu.make_async_copy(doT_hbm, doT_ref, sem_in.at[2])

    cp_x[0].start()
    cp_c[0].start()
    cp_c[1].start()
    tr_s[NO:256, :] = jnp.zeros((256 - NO, S), jnp.uint32)

    def fwd_a(cs):
        pt_s[0:2 * NE, cs] = _dg(fe_ref[...], a_s[0:H, cs], _NN)
        pt_s[2 * NE:2 * DFP, cs] = _dg(fo_ref[...], a_s[H:D, cs], _NN)

    def split_store(u, cs):
        a_s[0:H, cs] = (u[0:H] + u[H:D]).astype(bf16)
        a_s[H:D, cs] = (u[0:H] - u[H:D]).astype(bf16)

    def inv_b(cs):
        e = _dg(ge_ref[...], zt_s[0:2 * NE, cs], _NN)
        o = _dg(go_ref[...], zt_s[2 * NE:2 * DFP, cs], _NN)
        return jnp.concatenate([e + o, e - o], axis=0)

    def mid_f(si):
        r0, sl = _SLABS[si]
        rre, rim = _rows(r0)
        xs = [(pt_s[rre:rre + sl, s1 * R2:(s1 + 1) * R2],
               pt_s[rim:rim + sl, s1 * R2:(s1 + 1) * R2]) for s1 in range(R1)]
        ys = _fft_list(xs, False)
        rows = []
        for k1 in range(R1):
            re, im = ys[k1]
            if k1 > 0:
                c = tw_ref[k1:k1 + 1, :]
                sn = tw_ref[R1 + k1:R1 + k1 + 1, :]
                re, im = re * c - im * sn, re * sn + im * c
            rows.append(jnp.concatenate([re, im], axis=1))
        bb = jnp.concatenate(rows, axis=0).astype(bf16)
        return _dg(bb, mf_ref[...], _NN).reshape(R1, sl, 2 * R2)

    def mid_b(si, V):
        r0, sl = _SLABS[si]
        rre, rim = _rows(r0)
        C = _dg(V.reshape(R1 * sl, 2 * R2).astype(bf16), mi_ref[...], _NN)
        C = C.reshape(R1, sl, 2 * R2)
        xs = []
        for k1 in range(R1):
            re = C[k1, :, 0:R2]
            im = C[k1, :, R2:2 * R2]
            if k1 > 0:
                c = tw_ref[k1:k1 + 1, :]
                sn = tw_ref[R1 + k1:R1 + k1 + 1, :]
                re, im = re * c + im * sn, im * c - re * sn
            xs.append((re, im))
        zs = _fft_list(xs, True)
        for s1 in range(R1):
            zt_s[rre:rre + sl, s1 * R2:(s1 + 1) * R2] = zs[s1][0].astype(bf16)
            zt_s[rim:rim + sl, s1 * R2:(s1 + 1) * R2] = zs[s1][1].astype(bf16)

    def slab_rows(si):
        r0, sl = _SLABS[si]
        return slice(r0, r0 + sl)

    def freq_scale():
        r = jax.lax.broadcasted_iota(jnp.int32, (DFP, R2), 0)
        scale = jnp.where((r == 0) | (r == H // 2), 1.0, 2.0) * (1.0 / (S * D))
        return jnp.where((r <= H // 2) | (r >= NE), scale, 0.0).astype(f32)

    def ln1_chunk(c):
        cs = slice(c * CW, (c + 1) * CW)
        x = xT_ref[:, cs].astype(f32)
        m = jnp.mean(x, axis=0, keepdims=True)
        xc = x - m
        v = jnp.mean(xc * xc, axis=0, keepdims=True)
        r1 = jax.lax.rsqrt(v + EPS)
        n1 = xc * r1
        n1T_s[:, cs] = n1.astype(bf16)
        r1_s[:, cs] = r1
        split_store(n1, cs)
        fwd_a(cs)

    def wprep(c):
        scale = freq_scale()
        hi = jnp.uint32(0xFFFF0000)
        tr_s[0:NO, :] = pltpu.bitcast(wT_ref[c, 0:H, :], jnp.uint32)
        tr_s[NO:NO + 1, :] = pltpu.bitcast(wT_ref[c, H:DF, :].astype(f32), jnp.uint32) >> 16
        for q in range(2):
            wtmp_s[q] = tr_s[q * 128:(q + 1) * 128, :].T
        for k1 in range(R1):
            b0 = wtmp_s[0, pl.ds(k1, R2, stride=R1), :].T
            b1 = wtmp_s[1, pl.ds(k1, R2, stride=R1), :].T[0:NE - 128, :]
            u = jnp.concatenate([b0, b1], axis=0)
            cl = slice(c * R2, (c + 1) * R2)
            w_s[k1, 0:NE, cl] = pltpu.bitcast(u << 16, f32) * scale[0:NE]
            w_s[k1, NE:DFP, cl] = pltpu.bitcast(u[0:NO] & hi, f32) * scale[NE:DFP]

    NS = len(_SLABS)
    LEAD = LEAD_SLABS

    def f_store(si):
        x_s[:, slab_rows(si), :] = mid_f(si)

    def b_fwd(si):
        rs = slab_rows(si)
        xr = x_s[:, rs, 0:R2]
        xi = x_s[:, rs, R2:2 * R2]
        wr = w_s[:, rs, 0:R2]
        wi = w_s[:, rs, R2:2 * R2]
        mid_b(si, jnp.concatenate([xr * wr - xi * wi, xr * wi + xi * wr], axis=2))

    with _scope("ln1"):
        cp_x[0].wait()
        cp_c[0].wait()
        cp_c[1].wait()
        cp_x[1].start()
        ln1_chunk(0)
        cp_x[1].wait()
        cp_x[2].start()
        cp_x[3].start()
        ln1_chunk(1)
        cp_x[2].wait()
        for i in range(2, 5):
            cp_c[i].start()
        cp_wr.start()
        ln1_chunk(2)
        cp_x[3].wait()
        cp_wi.start()
        ln1_chunk(3)
        for i in range(2, 5):
            cp_c[i].wait()
        cp_wr.wait()
        for i in range(5, 7):
            cp_c[i].start()
        cp_do.start()

    with _scope("mid1"):
        wprep(0)
        for si in range(LEAD // 2):
            f_store(si)
        cp_wi.wait()
        for t in range(3):
            w_copy(0, 0, t).start()
        wprep(1)
        for si in range(LEAD // 2, LEAD):
            f_store(si)
        for si in range(NS):
            if si + LEAD < NS:
                f_store(si + LEAD)
            b_fwd(si)

    with _scope("ln2"):
        cp_c[5].wait()
        cp_c[6].wait()
        cp_do.wait()
        do_s[...] = doT_ref[...].T
        y_next = inv_b(slice(0, CW2))
        for c in range(NC2):
            cs = slice(c * CW2, (c + 1) * CW2)
            y = y_next
            if c + 1 < NC2:
                y_next = inv_b(slice((c + 1) * CW2, (c + 2) * CW2))
            h = xT_ref[:, cs].astype(f32) + y
            outT_s[:, cs] = h
            m = jnp.mean(h, axis=0, keepdims=True)
            hc = h - m
            v = jnp.mean(hc * hc, axis=0, keepdims=True)
            r2 = jax.lax.rsqrt(v + EPS)
            n2T = (hc * r2).astype(bf16)
            n2T_s[:, cs] = n2T
            r2_s[:, cs] = r2
            n2_s[cs, :] = n2T.T
        dn2T_s[...] = jnp.zeros_like(dn2T_s)

    def ffn_step(j, carry):
        slot = jax.lax.rem(j, 2)
        for t in range(3):
            w_copy(j, slot, t).wait()

        @pl.when(j + 1 < NF)
        def _():
            for t in range(3):
                w_copy(j + 1, 1 - slot, t).start()

        @pl.when(j >= 2)
        def _():
            for t in range(3):
                o_copy(j - 2, slot, t).wait()

        with _scope("ffn"):
            n2 = n2_s[...]
            wg = wbuf[slot, 0]
            wu = wbuf[slot, 1]
            wdT = wbuf[slot, 2]
            a = _dg(n2, wg, _NN)
            b = _dg(n2, wu, _NN)
            dgu = _dg(do_s[...], wdT, _NN)
            sig = jax.nn.sigmoid(a)
            g = a * sig
            gu = (g * b).astype(bf16)
            dgg = dgu * b
            db = (dgu * g).astype(bf16)
            da = (dgg * (sig * (1.0 + a * (1.0 - sig)))).astype(bf16)
            outT_s[...] += _dg(wdT, gu, _NT)
            dn2T_s[...] += _dg(wg, da, _NT) + _dg(wu, db, _NT)
            obuf[slot, 2] = _dg(doT_ref[...], gu, _NN).astype(bf16)
            obuf[slot, 0] = _dg(n2T_s[...], da, _NN).astype(bf16)
            obuf[slot, 1] = _dg(n2T_s[...], db, _NN).astype(bf16)
        for t in range(3):
            o_copy(j, slot, t).start()
        return carry

    jax.lax.fori_loop(0, NF, ffn_step, 0)

    cp_out = pltpu.make_async_copy(oT_ref, outT_hbm, sem_out.at[0])
    cp_dwr = pltpu.make_async_copy(dwT_ref.at[0], dwrT_hbm, sem_out.at[1])
    cp_dwi = pltpu.make_async_copy(dwT_ref.at[1], dwiT_hbm, sem_out.at[2])
    cp_dx = [pltpu.make_async_copy(dxT_ref.at[:, c * CW2:(c + 1) * CW2],
                                   dxT_hbm.at[:, c * CW2:(c + 1) * CW2], sem_dx.at[c])
             for c in range(NC2)]
    with _scope("ln2b"):
        for c in range(NC2):
            cs = slice(c * CW2, (c + 1) * CW2)
            dn2 = dn2T_s[:, cs]
            n2f = n2T_s[:, cs].astype(f32)
            c1 = jnp.mean(dn2, axis=0, keepdims=True)
            c2 = jnp.mean(dn2 * n2f, axis=0, keepdims=True)
            dh = doT_ref[:, cs].astype(f32) + r2_s[:, cs] * (dn2 - c1 - n2f * c2)
            oT_ref[:, cs] = outT_s[:, cs].astype(bf16)
            hT_s[:, cs] = dh
            split_store(dh, cs)
            if c > 0:
                fwd_a(slice((c - 1) * CW2, c * CW2))
        fwd_a(slice((NC2 - 1) * CW2, NC2 * CW2))
        cp_out.start()

    scale = freq_scale()

    def pw_bwd(G, rs):
        gr = G[:, :, 0:R2]
        gi = G[:, :, R2:2 * R2]
        xr = x_s[:, rs, 0:R2]
        xi = x_s[:, rs, R2:2 * R2]
        sc = scale[rs, :]
        x_s[:, rs, 0:R2] = (gr * xr + gi * xi) * sc
        x_s[:, rs, R2:2 * R2] = (gi * xr - gr * xi) * sc
        wr = w_s[:, rs, 0:R2]
        wi = w_s[:, rs, R2:2 * R2]
        return jnp.concatenate([gr * wr + gi * wi, gi * wr - gr * wi], axis=2)

    for jj in (NF - 2, NF - 1):
        for t in range(3):
            o_copy(jj, jj % 2, t).wait()
    with _scope("mid2"):
        for si in range(NS):
            mid_b(si, pw_bwd(mid_f(si), slab_rows(si)))
    cp_out.wait()

    with _scope("tail"):
        hi = jnp.uint32(0xFFFF0000)
        zpad = jnp.zeros((256 - NE, R2), jnp.uint32)
        zodd = jnp.zeros((NE - NO, R2), jnp.uint32)
        for c in range(2):
            cl = slice(c * R2, (c + 1) * R2)
            for k1 in range(R1):
                ev = x_s[k1, 0:NE, cl].astype(bf16).astype(f32)
                od = x_s[k1, NE:DFP, cl].astype(bf16).astype(f32)
                u = (pltpu.bitcast(ev, jnp.uint32) >> 16) | jnp.concatenate(
                    [pltpu.bitcast(od, jnp.uint32) & hi, zodd], axis=0)
                wtmp_s[0, pl.ds(k1, R2, stride=R1), :] = u[0:128].T
                wtmp_s[1, pl.ds(k1, R2, stride=R1), :] = jnp.concatenate(
                    [u[128:NE], zpad], axis=0).T
            for q in range(2):
                tr_s[q * 128:(q + 1) * 128, :] = wtmp_s[q].T
            dwT_ref[c, 0:H, :] = pltpu.bitcast(tr_s[0:NO, :], bf16)
            dwT_ref[c, H:DF, :] = pltpu.bitcast(tr_s[NO:NO + 1, :] << 16, f32).astype(bf16)
            (cp_dwr, cp_dwi)[c].start()
        d_next = inv_b(slice(0, CW2))
        for c in range(NC2):
            cs = slice(c * CW2, (c + 1) * CW2)
            dn1 = d_next
            if c + 1 < NC2:
                d_next = inv_b(slice((c + 1) * CW2, (c + 2) * CW2))
            n1f = n1T_s[:, cs].astype(f32)
            c1 = jnp.mean(dn1, axis=0, keepdims=True)
            c2 = jnp.mean(dn1 * n1f, axis=0, keepdims=True)
            dxT_ref[:, cs] = (hT_s[:, cs] + r1_s[:, cs] * (dn1 - c1 - n1f * c2)).astype(bf16)
            cp_dx[c].start()

    cp_dwr.wait()
    cp_dwi.wait()
    for c in range(NC2):
        cp_dx[c].wait()


@jax.jit
def pallas_sequential_preLN__spectral_gfnet__swiglu_ffn__prompt_kernel(
    A_x: jax.Array,
    A_w_r: jax.Array,
    A_w_i: jax.Array,
    B_x: jax.Array,
    B_w_gate: jax.Array,
    B_w_up: jax.Array,
    B_w_down: jax.Array,
    grad_out: jax.Array,
):
    xT = A_x.reshape(S, D).T
    doT = grad_out.reshape(S, D).T
    wrT = A_w_r.T
    wiT = A_w_i.T
    wdT = B_w_down.T
    bf = jnp.bfloat16
    f32 = jnp.float32
    fe, fo, mf, mi, tw = _const_tables()
    consts = [
        jnp.asarray(fe, dtype=bf), jnp.asarray(fo, dtype=bf),
        jnp.asarray(np.ascontiguousarray(fe.T), dtype=bf),
        jnp.asarray(np.ascontiguousarray(fo.T), dtype=bf),
        jnp.asarray(mf, dtype=bf), jnp.asarray(mi, dtype=bf),
        jnp.asarray(tw, dtype=f32),
    ]

    hbm = pl.BlockSpec(memory_space=pl.ANY)
    in_specs = [hbm] * 14
    out_specs = [hbm] * 7
    out_shape = [
        jax.ShapeDtypeStruct((D, S), bf), jax.ShapeDtypeStruct((D, S), bf),
        jax.ShapeDtypeStruct((DF, S), bf), jax.ShapeDtypeStruct((DF, S), bf),
        jax.ShapeDtypeStruct((D, F), bf), jax.ShapeDtypeStruct((D, F), bf),
        jax.ShapeDtypeStruct((D, F), bf),
    ]
    scratch = [pltpu.VMEM(c.shape, c.dtype) for c in consts] + [
        pltpu.VMEM((D, S), bf),
        pltpu.VMEM((D, S), bf),
        pltpu.VMEM((2, DF, S), bf),
        pltpu.VMEM((D, S), bf),
        pltpu.VMEM((D, S), bf),
        pltpu.VMEM((2, DF, S), bf),
        pltpu.VMEM((2, 3, D, TF), bf),
        pltpu.VMEM((2, 3, D, TF), bf),
        pltpu.VMEM((D, S), bf),
        pltpu.VMEM((1, S), f32),
        pltpu.VMEM((D, S), f32),
        pltpu.VMEM((D, S), bf),
        pltpu.VMEM((1, S), f32),
        pltpu.VMEM((S, D), bf),
        pltpu.VMEM((S, D), bf),
        pltpu.VMEM((D, S), f32),
        pltpu.VMEM((D, S), f32),
        pltpu.VMEM((D, S), bf),
        pltpu.VMEM((2 * DFP, S), f32),
        pltpu.VMEM((2 * DFP, S), bf),
        pltpu.VMEM((R1, DFP, 2 * R2), f32),
        pltpu.VMEM((R1, DFP, 2 * R2), f32),
        pltpu.VMEM((2, S, 128), jnp.uint32),
        pltpu.VMEM((256, S), jnp.uint32),
        pltpu.SemaphoreType.DMA((NC,)),
        pltpu.SemaphoreType.DMA((3,)),
        pltpu.SemaphoreType.DMA((7,)),
        pltpu.SemaphoreType.DMA((2, 3)),
        pltpu.SemaphoreType.DMA((2, 3)),
        pltpu.SemaphoreType.DMA((NC2,)),
        pltpu.SemaphoreType.DMA((3,)),
    ]
    outs = pl.pallas_call(
        _kernel,
        in_specs=in_specs,
        out_specs=out_specs,
        out_shape=out_shape,
        scratch_shapes=scratch,
        compiler_params=pltpu.CompilerParams(
            vmem_limit_bytes=120 * 1024 * 1024,
        ),
    )(xT, doT, wrT, wiT, B_w_gate, B_w_up, wdT, *consts)
    outT, dxT, dwrT, dwiT, dwg, dwu, dwdT = outs
    return (outT.T.reshape(1, S, D), dxT.T.reshape(1, S, D), dwrT.T, dwiT.T, dwg, dwu, dwdT.T)
```
